```python
import jax
import jax.numpy as jnp

def _softmax(x, axis=-1):
    return jax.nn.softmax(x, axis=axis)
def _gelu(x):
    return jax.nn.gelu(x, approximate=True)
def _silu(x):
    return jax.nn.silu(x)
def _sigmoid(x):
    return jax.nn.sigmoid(x)
def _layernorm(x, axis=-1, eps=1e-5):
    m = jnp.mean(x, axis=axis, keepdims=True)
    v = jnp.var(x, axis=axis, keepdims=True)
    return (x - m) / jnp.sqrt(v + eps)
def _scatter_add(tgt, idx, src, axis=0):
    return tgt.at[idx].add(src)
def _segment_sum(src, seg, n):
    return jax.ops.segment_sum(src, seg, n)
class _Rng:
    def __init__(self, key):
        self._k = key
    def _next(self):
        self._k, sub = jax.random.split(self._k)
        return sub
    def normal(self, shape):
        return jax.random.normal(self._next(), shape, dtype=jnp.bfloat16)
    def randint(self, lo, hi, shape):
        return jax.random.randint(self._next(), shape, lo, hi, dtype=jnp.int32)
    def uniform(self, shape, lo=0.0, hi=1.0):
        return jax.random.uniform(self._next(), shape, jnp.bfloat16, lo, hi)
    def permutation(self, n):
        return jax.random.permutation(self._next(), n)


kernel_name = 'gated_mix__sliding_local_dilated__glu_gated_geglu__prompt'

def setup_inputs():
    _rng = _Rng(jax.random.key(int.from_bytes(__import__("os").urandom(4), "little")))
    _w = (lambda a: (lambda t: t.astype(jnp.bfloat16) if jnp.issubdtype(t.dtype, jnp.floating) else t)(jnp.asarray(a)))
    def _A_setup():
        B, S, D = 1, 2048, 1024
        return {
            "x": _w((lambda *s: _rng.normal(s) * 0.05)(B, S, D)),
            "wqkv": _w((lambda *s: _rng.normal(s) * 0.05)(D, 3 * D)),
            "wo": _w((lambda *s: _rng.normal(s) * 0.05)(D, D)),
        }
    _A_in = _A_setup()

    def _B_setup():
        B, S, Dm, Df = 1, 2048, 1024, 3584
        return {
            "x": _w((lambda *s: _rng.normal(s) * 0.05)(B, S, Dm)),
            "w_gate": _w((lambda *s: _rng.normal(s) * 0.05)(Dm, Df) * (Dm ** -0.5)),
            "w_up": _w((lambda *s: _rng.normal(s) * 0.05)(Dm, Df) * (Dm ** -0.5)),
            "w_down": _w((lambda *s: _rng.normal(s) * 0.05)(Df, Dm) * (Df ** -0.5)),
        }
    _B_in = _B_setup()

    return {
        "A_x": _A_in["x"],
        "A_wqkv": _A_in["wqkv"],
        "A_wo": _A_in["wo"],
        "B_x": _B_in["x"],
        "B_w_gate": _B_in["w_gate"],
        "B_w_up": _B_in["w_up"],
        "B_w_down": _B_in["w_down"],
        "gate_w": _w((lambda *s: _rng.normal(s) * 0.05)(1024)),
    }

def reference(A_x, A_wqkv, A_wo, B_x, B_w_gate, B_w_up, B_w_down, gate_w):
    def _A_ref(x, wqkv, wo):
        B, S, D = x.shape
        H = 32; Dh = D // H
        W, dil = 8, 2
        qkv = (lambda x, *d: x.transpose(*d))((x @ wqkv).reshape(B, S, 3, H, Dh), 2, 0, 3, 1, 4)
        q, k, v = qkv[0], qkv[1], qkv[2]
        scale = Dh ** -0.5
        pos = jnp.arange(S)
        off = jnp.arange(W) * dil
        idx = pos[:, None] - off[None, :]
        mask = idx >= 0
        idx_c = jnp.where(mask, idx, 0).reshape(-1)
        kg = k[:, :, idx_c, :].reshape(B, H, S, W, Dh)
        vg = v[:, :, idx_c, :].reshape(B, H, S, W, Dh)
        logits = jnp.einsum("bhsd,bhswd->bhsw", q, kg) * scale
        logits = jnp.where(mask[None, None, :, :], logits, -1e9)
        attn = _softmax(logits, axis=-1)
        o = jnp.einsum("bhsw,bhswd->bhsd", attn, vg)
        return (lambda x, *d: x.transpose(*d))(o, 0, 2, 1, 3).reshape(B, S, D) @ wo

    def _B_ref(x, w_gate, w_up, w_down):
        g = jnp.einsum("bsd,df->bsf", x, w_gate)
        u = jnp.einsum("bsd,df->bsf", x, w_up)
        h = _gelu(g) * u
        return jnp.einsum("bsf,fd->bsd", h, w_down)

    x = A_x
    g = _sigmoid((x * gate_w).sum(-1, keepdims=True))
    a = _A_ref(x, A_wqkv, A_wo)
    b = _B_ref(x, B_w_gate, B_w_up, B_w_down)
    return g * a + (1 - g) * b
```

```python
import functools
import jax, jax.numpy as jnp
from jax.experimental import pallas as pl
from jax.experimental.pallas import tpu as pltpu

S, D, DF = 2048, 1024, 3584
H, DH, W, DIL = 32, 32, 8, 2
HALO = 16
NT = D // 128


def _butterfly(T, lane, reverse=False):
    T = list(T)
    stages = [(1, 16), (2, 8), (4, 4)]
    if reverse:
        stages = stages[::-1]
    for tb, g in stages:
        lower = (lane & g) == 0
        for j in range(NT):
            if j & tb:
                continue
            A, B = T[j], T[j + tb]
            T[j] = jnp.where(lower, A, pltpu.roll(B, g, 1))
            T[j + tb] = jnp.where(lower, pltpu.roll(A, 128 - g, 1), B)
    return T


def _make(tm=256, fc=256, qc=512, slab=16, fslab=24):
    nsteps = S // tm
    nchunk = DF // fc
    nq = 3 * D // qc
    nslab = tm // slab
    scale = DH ** -0.5
    ncopies = nq + 3 * nchunk + 1
    assert nchunk * fslab >= tm

    def kernel(xa_ref, xb_ref, gw_ref, wqkv_hbm, wo_hbm, wg_hbm, wu_hbm, wd_hbm, o_ref,
               wqkv_s, wo_s, wg_s, wu_s, wd_s, q_s, k_s, v_s, ob_s, raw_s, acc_s, sems):
        i = pl.program_id(0)

        def qkv_dma(c):
            return pltpu.make_async_copy(wqkv_hbm.at[:, pl.ds(c * qc, qc)], wqkv_s.at[c], sems.at[c])

        def g_dma(c):
            return pltpu.make_async_copy(wg_hbm.at[:, pl.ds(c * fc, fc)], wg_s.at[c], sems.at[nq + 3 * c])

        def u_dma(c):
            return pltpu.make_async_copy(wu_hbm.at[:, pl.ds(c * fc, fc)], wu_s.at[c], sems.at[nq + 3 * c + 1])

        def d_dma(c):
            return pltpu.make_async_copy(wd_hbm.at[pl.ds(c * fc, fc), :], wd_s.at[c], sems.at[nq + 3 * c + 2])

        def o_dma():
            return pltpu.make_async_copy(wo_hbm, wo_s, sems.at[ncopies - 1])

        def get_gate(xa):
            gl = jnp.sum(xa.astype(jnp.float32) * gw_ref[...].astype(jnp.float32), axis=-1, keepdims=True)
            return jax.nn.sigmoid(gl)

        def attn(r0, n, qv, gate_rows, mask_rows):
            lane_s = jax.lax.broadcasted_iota(jnp.int32, (n, 128), 1)
            L = []
            for w in range(W):
                f = None
                for t in range(NT):
                    p = qv[t] * k_s[t, pl.ds(HALO + r0 - DIL * w, n), :]
                    f = p if f is None else f + p
                for g in (1, 2):
                    sw = jnp.where((lane_s & g) == 0, pltpu.roll(f, 128 - g, 1), pltpu.roll(f, g, 1))
                    f = f + sw
                L.append(f)
            if mask_rows:
                row = jax.lax.broadcasted_iota(jnp.int32, (n, 128), 0) + (i * tm + r0)
                L = [L[0]] + [jnp.where(row >= DIL * w, L[w], -1e9) for w in range(1, W)]
            m = L[0]
            for w in range(1, W):
                m = jnp.maximum(m, L[w])
            E = [jnp.exp(L[w] - m) for w in range(W)]
            s = E[0]
            for w in range(1, W):
                s = s + E[w]
            r = gate_rows / s
            P = [E[w] * r for w in range(W)]
            o = []
            for t in range(NT):
                a = None
                for w in range(W):
                    p = P[w] * v_s[t, pl.ds(HALO + r0 - DIL * w, n), :]
                    a = p if a is None else a + p
                o.append(a)
            o = _butterfly(o, lane_s, reverse=True)
            for t in range(NT):
                ob_s[pl.ds(r0, n), t * 128:(t + 1) * 128] = o[t].astype(jnp.bfloat16)

        def first():
            for c in range(nq):
                qkv_dma(c).start()
            for c in range(nchunk):
                g_dma(c).start()
                u_dma(c).start()
                d_dma(c).start()
            o_dma().start()
            k_s[:, 0:HALO, :] = jnp.zeros((NT, HALO, 128), jnp.float32)
            v_s[:, 0:HALO, :] = jnp.zeros((NT, HALO, 128), jnp.float32)
            acc_s[...] = jnp.zeros((tm, D), jnp.float32)
            gate = get_gate(xa_ref[...])
            q_s[0] = jnp.broadcast_to(gate, (tm, 128))

            def qkv_body(c, carry):
                qkv_dma(c).wait()
                r = jnp.dot(xa_ref[...], wqkv_s[c], preferred_element_type=jnp.float32)
                for t in range(qc // 128):
                    raw_s[c * (qc // 128) + t] = r[:, t * 128:(t + 1) * 128]
                return carry

            jax.lax.fori_loop(0, nq, qkv_body, 0)

            def ffn_body(c, carry):
                g_dma(c).wait()
                u_dma(c).wait()
                d_dma(c).wait()
                r0 = pl.multiple_of(jnp.minimum(c * fslab, tm - fslab), 8)
                lane_s = jax.lax.broadcasted_iota(jnp.int32, (fslab, 128), 1)
                qv = _butterfly([raw_s[t, pl.ds(r0, fslab), :] for t in range(NT)], lane_s)
                qv = [x * scale for x in qv]
                kv = _butterfly([raw_s[NT + t, pl.ds(r0, fslab), :] for t in range(NT)], lane_s)
                vv = _butterfly([raw_s[2 * NT + t, pl.ds(r0, fslab), :] for t in range(NT)], lane_s)
                for t in range(NT):
                    k_s[t, pl.ds(HALO + r0, fslab), :] = kv[t]
                    v_s[t, pl.ds(HALO + r0, fslab), :] = vv[t]
                attn(r0, fslab, qv, q_s[0, pl.ds(r0, fslab), :], True)
                xb = xb_ref[...]
                omg = 1.0 - q_s[0, :, 0:1]
                g = jnp.dot(xb, wg_s[c], preferred_element_type=jnp.float32)
                u = jnp.dot(xb, wu_s[c], preferred_element_type=jnp.float32)
                h = (jax.nn.gelu(g, approximate=True) * u * omg).astype(jnp.bfloat16)
                acc_s[...] += jnp.dot(h, wd_s[c], preferred_element_type=jnp.float32)
                return carry

            jax.lax.fori_loop(0, nchunk, ffn_body, 0)
            o_dma().wait()
            o_ref[...] = (acc_s[...] + jnp.dot(ob_s[...], wo_s[...], preferred_element_type=jnp.float32)).astype(o_ref.dtype)

        def main():
            k_s[:, 0:HALO, :] = k_s[:, tm:tm + HALO, :]
            v_s[:, 0:HALO, :] = v_s[:, tm:tm + HALO, :]
            xa = xa_ref[...]
            xb = xb_ref[...]
            gate = get_gate(xa)
            lane = jax.lax.broadcasted_iota(jnp.int32, (tm, 128), 1)
            tiles = []
            for mat in range(3):
                raw = []
                for c in range(mat * nq // 3, (mat + 1) * nq // 3):
                    r = jnp.dot(xa, wqkv_s[c], preferred_element_type=jnp.float32)
                    raw += [r[:, t * 128:(t + 1) * 128] for t in range(qc // 128)]
                b = _butterfly(raw, lane)
                for t in range(NT):
                    if mat == 0:
                        q_s[t] = b[t] * scale
                    elif mat == 1:
                        k_s[t, HALO:HALO + tm, :] = b[t]
                    else:
                        v_s[t, HALO:HALO + tm, :] = b[t]

            lane_s = jax.lax.broadcasted_iota(jnp.int32, (slab, 128), 1)
            never = lane_s > (127 + i)
            omg = 1.0 - gate
            sc = [0] * nchunk
            for sb in range(nslab):
                sc[(sb * nchunk) // nslab] += 1
            nxt = 0
            acc = None
            for c in range(nchunk):
                g = jnp.dot(xb, wg_s[c], preferred_element_type=jnp.float32)
                for _ in range(sc[c]):
                    r0 = nxt * slab
                    qv = [jnp.where(never, g[0:slab, 0:128], q_s[t, r0:r0 + slab, :]) for t in range(NT)]
                    attn(r0, slab, qv, gate[r0:r0 + slab], False)
                    nxt += 1
                u = jnp.dot(xb, wu_s[c], preferred_element_type=jnp.float32)
                h = (jax.nn.gelu(g, approximate=True) * u * omg).astype(jnp.bfloat16)
                d = jnp.dot(h, wd_s[c], preferred_element_type=jnp.float32)
                acc = d if acc is None else acc + d
            acc = acc + jnp.dot(ob_s[...], wo_s[...], preferred_element_type=jnp.float32)
            o_ref[...] = acc.astype(o_ref.dtype)

        pl.when(i == 0)(first)
        pl.when(i > 0)(main)

    def resident(shape):
        return pl.BlockSpec(shape, lambda i: (0, 0), pipeline_mode=pl.Buffered(1))

    hbm = pl.BlockSpec(memory_space=pl.ANY)

    def fn(A_x, A_wqkv, A_wo, B_x, B_w_gate, B_w_up, B_w_down, gate_w):
        xa = A_x.reshape(S, D)
        xb = B_x.reshape(S, D)
        gw = gate_w.reshape(1, D)
        out = pl.pallas_call(
            kernel,
            grid=(nsteps,),
            in_specs=[
                pl.BlockSpec((tm, D), lambda i: (i, 0)),
                pl.BlockSpec((tm, D), lambda i: (i, 0)),
                resident((1, D)),
                hbm, hbm, hbm, hbm, hbm,
            ],
            out_specs=pl.BlockSpec((tm, D), lambda i: (i, 0)),
            out_shape=jax.ShapeDtypeStruct((S, D), jnp.bfloat16),
            scratch_shapes=[
                pltpu.VMEM((nq, D, qc), jnp.bfloat16),
                pltpu.VMEM((D, D), jnp.bfloat16),
                pltpu.VMEM((nchunk, D, fc), jnp.bfloat16),
                pltpu.VMEM((nchunk, D, fc), jnp.bfloat16),
                pltpu.VMEM((nchunk, fc, D), jnp.bfloat16),
                pltpu.VMEM((NT, tm, 128), jnp.float32),
                pltpu.VMEM((NT, HALO + tm, 128), jnp.float32),
                pltpu.VMEM((NT, HALO + tm, 128), jnp.float32),
                pltpu.VMEM((tm, D), jnp.bfloat16),
                pltpu.VMEM((3 * NT, tm, 128), jnp.float32),
                pltpu.VMEM((tm, D), jnp.float32),
                pltpu.SemaphoreType.DMA((ncopies,)),
            ],
            compiler_params=pltpu.CompilerParams(
                dimension_semantics=("arbitrary",), vmem_limit_bytes=110 * 1024 * 1024),
            name="fused",
        )(xa, xb, gw, A_wqkv, A_wo, B_w_gate, B_w_up, B_w_down)
        return out.reshape(1, S, D)

    return fn


_FN = _make()


@jax.jit
def pallas_gated_mix__sliding_local_dilated__glu_gated_geglu__prompt_kernel(
    A_x: jax.Array,
    A_wqkv: jax.Array,
    A_wo: jax.Array,
    B_x: jax.Array,
    B_w_gate: jax.Array,
    B_w_up: jax.Array,
    B_w_down: jax.Array,
    gate_w: jax.Array,
):
    return _FN(A_x, A_wqkv, A_wo, B_x, B_w_gate, B_w_up, B_w_down, gate_w)
```

```python
import jax
import jax.numpy as jnp
from jax.experimental import pallas as pl
from jax.experimental.pallas import tpu as pltpu

S, D, DF = 2048, 1024, 3584
DH, W, DIL = 32, 8, 2
HALO = 16
NT = D // 128
LOG2E = 1.4426950408889634

TM = 256
FC = 256
QC = 512
SLAB = 8
NSTEPS = S // TM
NCHUNK = DF // FC
NQ = 3 * D // QC
NSLAB = TM // SLAB
KR = HALO + TM + 8

SEM_GW, SEM_XA, SEM_Q = 0, 1, 1 + NSTEPS
SEM_XB = SEM_Q + NQ
SEM_G, SEM_U, SEM_D, SEM_O = SEM_XB + 1, SEM_XB + 2, SEM_XB + 3, SEM_XB + 4
NSEMS = SEM_O + 1


def _butterfly(tiles, lane, reverse=False):
    t = list(tiles)
    stages = [(1, 16), (2, 8), (4, 4)]
    if reverse:
        stages = stages[::-1]
    for tb, g in stages:
        lower = (lane & g) == 0
        for j in range(NT):
            if j & tb:
                continue
            a, b = t[j], t[j + tb]
            t[j] = jnp.where(lower, a, pltpu.roll(b, g, 1))
            t[j + tb] = jnp.where(lower, pltpu.roll(a, 128 - g, 1), b)
    return t


def _recip(s):
    r = pl.reciprocal(s, approx=True)
    return r * (2.0 - s * r)


def _kernel(xa_hbm, xb_hbm, gw_hbm, wqkv_hbm, wo_hbm, wg_hbm, wu_hbm, wd_hbm, o_ref,
            xa_s, xb_s, gw_s, wqkv_s, wo_s, wg_s, wu_s, wd_s, qkv_s, kc_s, ob_s, sems):
    i = pl.program_id(0)
    bf = jnp.bfloat16
    f32 = jnp.float32

    def asbf(v):
        return pltpu.bitcast(v, bf)

    def xa_dma(j):
        return pltpu.make_async_copy(xa_hbm.at[pl.ds(j * TM, TM), :],
                                     xa_s.bitcast(bf).at[pl.ds(j * TM, TM), :], sems.at[SEM_XA + j])

    def qkv_dma(c):
        return pltpu.make_async_copy(wqkv_hbm.at[:, pl.ds(c * QC, QC)], wqkv_s.bitcast(bf).at[c],
                                     sems.at[SEM_Q + c])

    rest = [
        pltpu.make_async_copy(gw_hbm, gw_s, sems.at[SEM_GW]),
        pltpu.make_async_copy(xb_hbm, xb_s.bitcast(bf), sems.at[SEM_XB]),
        pltpu.make_async_copy(wg_hbm, wg_s.bitcast(bf), sems.at[SEM_G]),
        pltpu.make_async_copy(wu_hbm, wu_s.bitcast(bf), sems.at[SEM_U]),
        pltpu.make_async_copy(wd_hbm, wd_s.bitcast(bf), sems.at[SEM_D]),
        pltpu.make_async_copy(wo_hbm, wo_s.bitcast(bf), sems.at[SEM_O]),
    ]

    @pl.when(i == 0)
    def _():
        xa_dma(0).start()
        for c in range(NQ):
            qkv_dma(c).start()
        for j in range(1, NSTEPS):
            xa_dma(j).start()
        for cp in rest:
            cp.start()
        kc_s[:, TM:TM + 24, :] = jnp.zeros((8 * NT, 24, 128), f32)
        xa_dma(0).wait()

        def first_block(c, carry):
            qkv_dma(c).wait()
            r = jnp.dot(asbf(xa_s[0:TM // 2, :]), asbf(wqkv_s[c]), preferred_element_type=f32)
            for t in range(QC // 128):
                qkv_s[c * (QC // 128) + t, 0:TM, :] = r[:, t * 128:(t + 1) * 128]
            return carry

        jax.lax.fori_loop(0, NQ, first_block, 0)

        def other_blocks(j, carry):
            xa_dma(j).wait()
            row0 = pl.multiple_of(j * TM, TM)
            xa = asbf(xa_s[pl.ds(pl.multiple_of(j * (TM // 2), TM // 2), TM // 2), :])
            for c in range(NQ):
                r = jnp.dot(xa, asbf(wqkv_s[c]), preferred_element_type=f32)
                for t in range(QC // 128):
                    qkv_s[c * (QC // 128) + t, pl.ds(row0, TM), :] = r[:, t * 128:(t + 1) * 128]
            return carry

        jax.lax.fori_loop(1, NSTEPS, other_blocks, 0)
        for cp in rest:
            cp.wait()

    row0 = pl.multiple_of(i * TM, TM)
    kc_s[:, 0:24, :] = kc_s[:, TM:TM + 24, :]
    hrow0 = pl.multiple_of(i * (TM // 2), TM // 2)
    xb = asbf(xb_s[pl.ds(hrow0, TM // 2), :])
    xa = asbf(xa_s[pl.ds(hrow0, TM // 2), :])
    gw = gw_s[...].astype(f32).reshape(1, D)
    gl = jnp.sum(xa.astype(f32) * gw, axis=-1, keepdims=True)
    gate = 0.5 * jnp.tanh(0.5 * gl) + 0.5
    omg = 1.0 - gate
    n = SLAB
    lane = jax.lax.broadcasted_iota(jnp.int32, (n, 128), 1)
    lane_h = jax.lax.broadcasted_iota(jnp.int32, (n // 2, 128), 1)
    never = lane > (127 + i)

    def tie(x, dep):
        return jnp.where(never, dep, x)

    def window(arr, t, w, r0):
        a, b = w % 4, w // 4
        return kc_s[(arr * 4 + a) * NT + t, pl.ds(HALO + r0 - 8 * b, n), :]

    def slab(r0, dep):
        base = row0 + r0
        for arr in range(2):
            bv = _butterfly([tie(qkv_s[(1 + arr) * NT + t, pl.ds(base, n), :], dep) for t in range(NT)], lane)
            for t in range(NT):
                for a in range(4):
                    kc_s[(arr * 4 + a) * NT + t, pl.ds(HALO + r0 + DIL * a, n), :] = bv[t]
        qv = _butterfly([tie(qkv_s[t, pl.ds(base, n), :], dep) for t in range(NT)], lane)
        logits = []
        for w in range(W):
            f = None
            for t in range(NT):
                p = qv[t] * window(0, t, w, r0)
                f = p if f is None else f + p
            for g in (1, 2):
                f = f + jnp.where((lane & g) == 0, pltpu.roll(f, 128 - g, 1), pltpu.roll(f, g, 1))
            logits.append(f)
        if r0 < HALO:
            row = jax.lax.broadcasted_iota(jnp.int32, (n, 128), 0) + (row0 + r0)
            logits = [logits[0]] + [jnp.where(row >= DIL * w, logits[w], -1e9) for w in range(1, W)]
        m = logits[0]
        for w in range(1, W):
            m = jnp.maximum(m, logits[w])
        e = [jnp.exp2((logits[w] - m) * (DH ** -0.5 * LOG2E)) for w in range(W)]
        s = e[0]
        for w in range(1, W):
            s = s + e[w]
        r = gate[r0:r0 + n] * _recip(s)
        p = [e[w] * r for w in range(W)]
        o = []
        for t in range(NT):
            acc_o = None
            for w in range(W):
                x = p[w] * window(1, t, w, r0)
                acc_o = x if acc_o is None else acc_o + x
            o.append(acc_o)
        ou = _butterfly([pltpu.bitcast(x.astype(bf), jnp.uint32) for x in o], lane_h, reverse=True)
        for t in range(NT):
            ob_s[r0 // 2:(r0 + n) // 2, t * 128:(t + 1) * 128] = ou[t]

    points = [(c, k) for c in range(NCHUNK) for k in "gud"]
    assign = {}
    for sb in range(NSLAB):
        assign.setdefault(points[(sb * len(points)) // NSLAB], []).append(sb)

    def run_slabs(c, k, m):
        for sb in assign.get((c, k), []):
            slab(sb * n, m[0:n, 0:128])

    acc = None
    for c in range(NCHUNK):
        g = jnp.dot(xb, asbf(wg_s[:, c * FC:(c + 1) * FC]), preferred_element_type=f32)
        run_slabs(c, "g", g)
        u = jnp.dot(xb, asbf(wu_s[:, c * FC:(c + 1) * FC]), preferred_element_type=f32)
        run_slabs(c, "u", u)
        h = (jax.nn.gelu(g, approximate=True) * u * omg).astype(bf)
        d = jnp.dot(h, asbf(wd_s[c * FC // 2:(c + 1) * FC // 2, :]), preferred_element_type=f32)
        run_slabs(c, "d", d)
        acc = d if acc is None else acc + d
    acc = acc + jnp.dot(asbf(ob_s[...]), asbf(wo_s[...]), preferred_element_type=f32)
    o_ref[...] = acc.astype(o_ref.dtype)


@jax.jit
def pallas_gated_mix__sliding_local_dilated__glu_gated_geglu__prompt_kernel(
    A_x: jax.Array,
    A_wqkv: jax.Array,
    A_wo: jax.Array,
    B_x: jax.Array,
    B_w_gate: jax.Array,
    B_w_up: jax.Array,
    B_w_down: jax.Array,
    gate_w: jax.Array,
):
    hbm = pl.BlockSpec(memory_space=pl.ANY)
    u32 = jnp.uint32
    out = pl.pallas_call(
        _kernel,
        grid=(NSTEPS,),
        in_specs=[hbm] * 8,
        out_specs=pl.BlockSpec((TM, D), lambda i: (i, 0)),
        out_shape=jax.ShapeDtypeStruct((S, D), jnp.bfloat16),
        scratch_shapes=[
            pltpu.VMEM((S // 2, D), u32),
            pltpu.VMEM((S // 2, D), u32),
            pltpu.VMEM((D,), jnp.bfloat16),
            pltpu.VMEM((NQ, D // 2, QC), u32),
            pltpu.VMEM((D // 2, D), u32),
            pltpu.VMEM((D // 2, DF), u32),
            pltpu.VMEM((D // 2, DF), u32),
            pltpu.VMEM((DF // 2, D), u32),
            pltpu.VMEM((3 * NT, S, 128), jnp.float32),
            pltpu.VMEM((8 * NT, KR, 128), jnp.float32),
            pltpu.VMEM((TM // 2, D), u32),
            pltpu.SemaphoreType.DMA((NSEMS,)),
        ],
        compiler_params=pltpu.CompilerParams(
            dimension_semantics=("arbitrary",), vmem_limit_bytes=120 * 1024 * 1024),
        name="fused",
    )(A_x.reshape(S, D), B_x.reshape(S, D), gate_w, A_wqkv, A_wo, B_w_gate, B_w_up, B_w_down)
    return out.reshape(1, S, D)
```

```python
import jax
import jax.numpy as jnp
from jax.experimental import pallas as pl
from jax.experimental.pallas import tpu as pltpu

S, D, DF = 2048, 1024, 3584
DH, W, DIL = 32, 8, 2
HALO = 16
NT = D // 128
LOG2E = 1.4426950408889634

TM = 256
FC = 256
QC = 512
SLAB = 8
NSTEPS = S // TM
NCHUNK = DF // FC
NQ = 3 * D // QC
NSLAB = TM // SLAB
KR = HALO + TM + 8

QT = QC // 128
OG = 2
OW = D // OG
PIECES = [(0, 128), (128, 128), (256, QC - 256)]

SEM_GW, SEM_XA = 0, 1
SEM_P = SEM_XA + NSTEPS
SEM_Q = SEM_P + len(PIECES)
SEM_G = SEM_Q + NQ
SEM_U, SEM_D, SEM_O = SEM_G + 1, SEM_G + 2, SEM_G + 3
SEM_OUT = SEM_O + 1
NSEMS = SEM_OUT + 2 * OG


def _butterfly(tiles, lane, reverse=False):
    t = list(tiles)
    stages = [(1, 16), (2, 8), (4, 4)]
    if reverse:
        stages = stages[::-1]
    for tb, g in stages:
        lower = (lane & g) == 0
        for j in range(NT):
            if j & tb:
                continue
            a, b = t[j], t[j + tb]
            t[j] = jnp.where(lower, a, pltpu.roll(b, g, 1))
            t[j + tb] = jnp.where(lower, pltpu.roll(a, 128 - g, 1), b)
    return t


def _recip(s):
    r = pl.reciprocal(s, approx=True)
    return r * (2.0 - s * r)


def _kernel(xa_hbm, gw_hbm, wqkv_hbm, wo_hbm, wg_hbm, wu_hbm, wd_hbm, o_hbm,
            xa_s, gw_s, wqkv_s, wo_s, wg_s, wu_s, wd_s, qkv_s, kc_s, ob_s, obuf, sems):
    i = pl.program_id(0)
    bf = jnp.bfloat16
    f32 = jnp.float32

    def asbf(v):
        return pltpu.bitcast(v, bf)

    def xa_dma(j):
        return pltpu.make_async_copy(xa_hbm.at[pl.ds(j * TM, TM), :],
                                     xa_s.bitcast(bf).at[pl.ds(j * TM, TM), :], sems.at[SEM_XA + j])

    def piece_dma(p):
        c0, cw = PIECES[p]
        return pltpu.make_async_copy(wqkv_hbm.at[:, pl.ds(c0, cw)],
                                     wqkv_s.bitcast(bf).at[0, :, pl.ds(c0, cw)], sems.at[SEM_P + p])

    def qkv_dma(c):
        return pltpu.make_async_copy(wqkv_hbm.at[:, pl.ds(c * QC, QC)], wqkv_s.bitcast(bf).at[c],
                                     sems.at[SEM_Q + c])

    def out_dma(step, g):
        slot = step % 2
        return pltpu.make_async_copy(obuf.at[slot, :, pl.ds(g * OW, OW)],
                                     o_hbm.at[pl.ds(step * TM, TM), pl.ds(g * OW, OW)],
                                     sems.at[SEM_OUT + slot * OG + g])

    rest = [
        pltpu.make_async_copy(gw_hbm, gw_s, sems.at[SEM_GW]),
        pltpu.make_async_copy(wg_hbm, wg_s.bitcast(bf), sems.at[SEM_G]),
        pltpu.make_async_copy(wu_hbm, wu_s.bitcast(bf), sems.at[SEM_U]),
        pltpu.make_async_copy(wd_hbm, wd_s.bitcast(bf), sems.at[SEM_D]),
        pltpu.make_async_copy(wo_hbm, wo_s.bitcast(bf), sems.at[SEM_O]),
    ]

    def proj(row_lo, nrows, c, c0, cw):
        r = jnp.dot(asbf(xa_s[row_lo // 2:(row_lo + nrows) // 2, :]), asbf(wqkv_s[c, :, c0:c0 + cw]),
                    preferred_element_type=f32)
        for t in range(cw // 128):
            qkv_s[c * QT + c0 // 128 + t, row_lo:row_lo + nrows, :] = r[:, t * 128:(t + 1) * 128]

    @pl.when(i == 0)
    def _():
        xa_dma(0).start()
        piece_dma(0).start()
        xa_dma(1).start()
        piece_dma(1).start()
        piece_dma(2).start()
        for c in range(1, NQ):
            qkv_dma(c).start()
        for j in range(2, NSTEPS):
            xa_dma(j).start()
        for cp in rest:
            cp.start()
        kc_s[:, TM:TM + 24, :] = jnp.zeros((8 * NT, 24, 128), f32)

        xa_dma(0).wait()
        piece_dma(0).wait()
        proj(0, TM, 0, 0, 128)
        xa_dma(1).wait()
        proj(TM, TM, 0, 0, 128)
        piece_dma(1).wait()
        proj(0, 2 * TM, 0, 128, 128)
        piece_dma(2).wait()
        proj(0, 2 * TM, 0, 256, QC - 256)

        def first_blocks(c, carry):
            qkv_dma(c).wait()
            proj(0, 2 * TM, c, 0, QC)
            return carry

        jax.lax.fori_loop(1, NQ, first_blocks, 0)

        def other_blocks(j, carry):
            xa_dma(j).wait()
            row0 = pl.multiple_of(j * TM, TM)
            xa = asbf(xa_s[pl.ds(pl.multiple_of(j * (TM // 2), TM // 2), TM // 2), :])
            for c in range(NQ):
                r = jnp.dot(xa, asbf(wqkv_s[c]), preferred_element_type=f32)
                for t in range(QT):
                    qkv_s[c * QT + t, pl.ds(row0, TM), :] = r[:, t * 128:(t + 1) * 128]
            return carry

        jax.lax.fori_loop(2, NSTEPS, other_blocks, 0)
        for cp in rest:
            cp.wait()

    @pl.when(i >= 2)
    def _():
        for g in range(OG):
            out_dma(i - 2, g).wait()

    row0 = pl.multiple_of(i * TM, TM)
    kc_s[:, 0:24, :] = kc_s[:, TM:TM + 24, :]
    hrow0 = pl.multiple_of(i * (TM // 2), TM // 2)
    xa = asbf(xa_s[pl.ds(hrow0, TM // 2), :])
    gw = gw_s[...].astype(f32).reshape(1, D)
    gl = jnp.sum(xa.astype(f32) * gw, axis=-1, keepdims=True)
    gate = 0.5 * jnp.tanh(0.5 * gl) + 0.5
    omg = 1.0 - gate
    n = SLAB
    lane = jax.lax.broadcasted_iota(jnp.int32, (n, 128), 1)
    lane_h = jax.lax.broadcasted_iota(jnp.int32, (n // 2, 128), 1)
    never = lane > (127 + i)

    def tie(x, dep):
        return jnp.where(never, dep, x)

    def window(arr, t, w, r0):
        a, b = w % 4, w // 4
        return kc_s[(arr * 4 + a) * NT + t, pl.ds(HALO + r0 - 8 * b, n), :]

    def slab(r0, dep):
        base = row0 + r0
        for arr in range(2):
            bv = _butterfly([tie(qkv_s[(1 + arr) * NT + t, pl.ds(base, n), :], dep) for t in range(NT)], lane)
            for t in range(NT):
                for a in range(4):
                    kc_s[(arr * 4 + a) * NT + t, pl.ds(HALO + r0 + DIL * a, n), :] = bv[t]
        qv = _butterfly([tie(qkv_s[t, pl.ds(base, n), :], dep) for t in range(NT)], lane)
        logits = []
        for w in range(W):
            f = None
            for t in range(NT):
                p = qv[t] * window(0, t, w, r0)
                f = p if f is None else f + p
            for g in (1, 2):
                f = f + jnp.where((lane & g) == 0, pltpu.roll(f, 128 - g, 1), pltpu.roll(f, g, 1))
            logits.append(f)
        if r0 < HALO:
            row = jax.lax.broadcasted_iota(jnp.int32, (n, 128), 0) + (row0 + r0)
            logits = [logits[0]] + [jnp.where(row >= DIL * w, logits[w], -1e9) for w in range(1, W)]
        m = logits[0]
        for w in range(1, W):
            m = jnp.maximum(m, logits[w])
        e = [jnp.exp2((logits[w] - m) * (DH ** -0.5 * LOG2E)) for w in range(W)]
        s = e[0]
        for w in range(1, W):
            s = s + e[w]
        r = gate[r0:r0 + n] * _recip(s)
        p = [e[w] * r for w in range(W)]
        o = []
        for t in range(NT):
            acc_o = None
            for w in range(W):
                x = p[w] * window(1, t, w, r0)
                acc_o = x if acc_o is None else acc_o + x
            o.append(acc_o)
        ou = _butterfly([pltpu.bitcast(x.astype(bf), jnp.uint32) for x in o], lane_h, reverse=True)
        for t in range(NT):
            ob_s[r0 // 2:(r0 + n) // 2, t * 128:(t + 1) * 128] = ou[t]

    points = [(c, k) for c in range(NCHUNK) for k in "gud"]
    assign = {}
    for sb in range(NSLAB):
        assign.setdefault(points[(sb * len(points)) // NSLAB], []).append(sb)

    def run_slabs(c, k, m):
        for sb in assign.get((c, k), []):
            slab(sb * n, m[0:n, 0:128])

    acc = None
    for c in range(NCHUNK):
        g = jnp.dot(xa, asbf(wg_s[:, c * FC:(c + 1) * FC]), preferred_element_type=f32)
        run_slabs(c, "g", g)
        u = jnp.dot(xa, asbf(wu_s[:, c * FC:(c + 1) * FC]), preferred_element_type=f32)
        run_slabs(c, "u", u)
        h = (jax.nn.gelu(g, approximate=True) * u * omg).astype(bf)
        d = jnp.dot(h, asbf(wd_s[c * FC // 2:(c + 1) * FC // 2, :]), preferred_element_type=f32)
        run_slabs(c, "d", d)
        acc = d if acc is None else acc + d
    ob = asbf(ob_s[...])
    slot = i % 2
    for g in range(OG):
        res = acc[:, g * OW:(g + 1) * OW] + jnp.dot(ob, asbf(wo_s[:, g * OW:(g + 1) * OW]),
                                                     preferred_element_type=f32)
        obuf[slot, :, g * OW:(g + 1) * OW] = res.astype(bf)
        out_dma(i, g).start()

    @pl.when(i == NSTEPS - 1)
    def _():
        for g in range(OG):
            out_dma(i - 1, g).wait()
        for g in range(OG):
            out_dma(i, g).wait()


@jax.jit
def pallas_gated_mix__sliding_local_dilated__glu_gated_geglu__prompt_kernel(
    A_x: jax.Array,
    A_wqkv: jax.Array,
    A_wo: jax.Array,
    B_x: jax.Array,
    B_w_gate: jax.Array,
    B_w_up: jax.Array,
    B_w_down: jax.Array,
    gate_w: jax.Array,
):
    del B_x
    hbm = pl.BlockSpec(memory_space=pl.ANY)
    u32 = jnp.uint32
    out = pl.pallas_call(
        _kernel,
        grid=(NSTEPS,),
        in_specs=[hbm] * 7,
        out_specs=hbm,
        out_shape=jax.ShapeDtypeStruct((S, D), jnp.bfloat16),
        scratch_shapes=[
            pltpu.VMEM((S // 2, D), u32),
            pltpu.VMEM((D,), jnp.bfloat16),
            pltpu.VMEM((NQ, D // 2, QC), u32),
            pltpu.VMEM((D // 2, D), u32),
            pltpu.VMEM((D // 2, DF), u32),
            pltpu.VMEM((D // 2, DF), u32),
            pltpu.VMEM((DF // 2, D), u32),
            pltpu.VMEM((3 * NT, S, 128), jnp.float32),
            pltpu.VMEM((8 * NT, KR, 128), jnp.float32),
            pltpu.VMEM((TM // 2, D), u32),
            pltpu.VMEM((2, TM, D), jnp.bfloat16),
            pltpu.SemaphoreType.DMA((NSEMS,)),
        ],
        compiler_params=pltpu.CompilerParams(
            dimension_semantics=("arbitrary",), vmem_limit_bytes=120 * 1024 * 1024),
        name="fused",
    )(A_x.reshape(S, D), gate_w, A_wqkv, A_wo, B_w_gate, B_w_up, B_w_down)
    return out.reshape(1, S, D)
```

```python
import jax
import jax.numpy as jnp
from jax.experimental import pallas as pl
from jax.experimental.pallas import tpu as pltpu

S, D, DF = 2048, 1024, 3584
DH, W, DIL = 32, 8, 2
HALO = 16
NT = D // 128
LOG2E = 1.4426950408889634

TM = 256
FC = 256
QC = 512
SLAB = 8
NSTEPS = S // TM
NCHUNK = DF // FC
NQ = 3 * D // QC
NSLAB = TM // SLAB
KR = HALO + TM + 8

QT = QC // 128
OG = 8
OW = D // OG
PIECES = [(0, 128), (128, 128), (256, QC - 256)]

SEM_X0, SEM_X1, SEM_XR, SEM_W = 0, 1, 2, 3
SEM_P = 4
SEM_Q = SEM_P + len(PIECES) - 1
SEM_OUT = SEM_Q + NQ
NSEMS = SEM_OUT + 2


def _butterfly(tiles, lane, reverse=False):
    t = list(tiles)
    stages = [(1, 16), (2, 8), (4, 4)]
    if reverse:
        stages = stages[::-1]
    for tb, g in stages:
        lower = (lane & g) == 0
        for j in range(NT):
            if j & tb:
                continue
            a, b = t[j], t[j + tb]
            t[j] = jnp.where(lower, a, pltpu.roll(b, g, 1))
            t[j + tb] = jnp.where(lower, pltpu.roll(a, 128 - g, 1), b)
    return t


def _recip(s):
    r = pl.reciprocal(s, approx=True)
    return r * (2.0 - s * r)


def _kernel(xa_hbm, gw_hbm, wqkv_hbm, wo_hbm, wg_hbm, wu_hbm, wd_hbm, o_hbm,
            xa_s, gw_s, wqkv_s, wo_s, wg_s, wu_s, wd_s, qkv_s, kc_s, ob_s, obuf, sems):
    i = pl.program_id(0)
    bf = jnp.bfloat16
    f32 = jnp.float32

    def asbf(v):
        return pltpu.bitcast(v, bf)

    def xa_dma(j):
        return pltpu.make_async_copy(xa_hbm.at[pl.ds(j * TM, TM), :],
                                     xa_s.at[pl.ds(j * TM, TM), :], sems.at[min(j, SEM_XR)])

    def piece_dma(p):
        c0, cw = PIECES[p]
        return pltpu.make_async_copy(wqkv_hbm.at[:, pl.ds(c0, cw)],
                                     wqkv_s.at[0, :, pl.ds(c0, cw)], sems.at[SEM_P + p])

    def qkv_dma(c):
        return pltpu.make_async_copy(wqkv_hbm.at[:, pl.ds(c * QC, QC)], wqkv_s.at[c],
                                     sems.at[SEM_Q + c])

    def out_dma(step, g):
        slot = step % 2
        return pltpu.make_async_copy(obuf.at[slot, :, pl.ds(g * OW, OW)],
                                     o_hbm.at[pl.ds(step * TM, TM), pl.ds(g * OW, OW)],
                                     sems.at[SEM_OUT + slot])

    rest = [
        pltpu.make_async_copy(gw_hbm, gw_s, sems.at[SEM_W]),
        pltpu.make_async_copy(wg_hbm, wg_s, sems.at[SEM_W]),
        pltpu.make_async_copy(wu_hbm, wu_s, sems.at[SEM_W]),
        pltpu.make_async_copy(wd_hbm, wd_s, sems.at[SEM_W]),
        pltpu.make_async_copy(wo_hbm, wo_s, sems.at[SEM_W]),
    ]

    def proj(row_lo, nrows, c, c0, cw):
        r = jnp.dot(xa_s[row_lo:row_lo + nrows, :], wqkv_s[c, :, c0:c0 + cw],
                    preferred_element_type=f32)
        for t in range(cw // 128):
            qkv_s[c * QT + c0 // 128 + t, row_lo:row_lo + nrows, :] = r[:, t * 128:(t + 1) * 128]

    @pl.when(i == 0)
    def _():
        xa_dma(0).start()
        piece_dma(0).start()
        piece_dma(1).start()
        xa_dma(1).start()
        piece_dma(2).start()
        for c in range(1, NQ):
            qkv_dma(c).start()
        for j in range(2, NSTEPS):
            xa_dma(j).start()
        for cp in rest:
            cp.start()
        kc_s[:, TM:TM + 24, :] = jnp.zeros((8 * NT, 24, 128), f32)

        xa_dma(0).wait()
        piece_dma(0).wait()
        proj(0, TM, 0, 0, 128)
        piece_dma(1).wait()
        proj(0, TM, 0, 128, 128)
        xa_dma(1).wait()
        proj(TM, TM, 0, 0, 256)
        piece_dma(2).wait()
        proj(0, 2 * TM, 0, 256, QC - 256)

        def first_blocks(c, carry):
            qkv_dma(c).wait()
            proj(0, 2 * TM, c, 0, QC)
            return carry

        jax.lax.fori_loop(1, NQ, first_blocks, 0)

        for j in range(2, NSTEPS):
            xa_dma(j).wait()

        def other_blocks(j, carry):
            row0 = pl.multiple_of(j * TM, TM)
            xa = xa_s[pl.ds(row0, TM), :]
            for c in range(NQ):
                r = jnp.dot(xa, wqkv_s[c], preferred_element_type=f32)
                for t in range(QT):
                    qkv_s[c * QT + t, pl.ds(row0, TM), :] = r[:, t * 128:(t + 1) * 128]
            return carry

        jax.lax.fori_loop(2, NSTEPS, other_blocks, 0)
        for cp in rest:
            cp.wait()

    @pl.when(i >= 2)
    def _():
        for g in range(OG):
            out_dma(i - 2, g).wait()

    row0 = pl.multiple_of(i * TM, TM)
    kc_s[:, 0:24, :] = kc_s[:, TM:TM + 24, :]
    xa = xa_s[pl.ds(row0, TM), :]
    gw = gw_s[...].astype(f32).reshape(1, D)
    gl = jnp.sum(xa.astype(f32) * gw, axis=-1, keepdims=True)
    gate = 0.5 * jnp.tanh(0.5 * gl) + 0.5
    omg = 1.0 - gate
    n = SLAB
    lane = jax.lax.broadcasted_iota(jnp.int32, (n, 128), 1)
    lane_h = jax.lax.broadcasted_iota(jnp.int32, (n // 2, 128), 1)
    never = lane > (127 + i)

    def tie(x, dep):
        return jnp.where(never, dep, x)

    def window(arr, t, w, r0):
        a, b = w % 4, w // 4
        return kc_s[(arr * 4 + a) * NT + t, pl.ds(HALO + r0 - 8 * b, n), :]

    def slab(r0, deps):
        base = row0 + r0
        for arr in range(2):
            bv = _butterfly([tie(qkv_s[(1 + arr) * NT + t, pl.ds(base, n), :], deps[arr]) for t in range(NT)], lane)
            for t in range(NT):
                for a in range(4):
                    kc_s[(arr * 4 + a) * NT + t, pl.ds(HALO + r0 + DIL * a, n), :] = bv[t]
        qv = _butterfly([tie(qkv_s[t, pl.ds(base, n), :], deps[2]) for t in range(NT)], lane)
        logits = []
        for w in range(W):
            f = None
            for t in range(NT):
                p = qv[t] * window(0, t, w, r0)
                f = p if f is None else f + p
            for g in (1, 2):
                f = f + jnp.where((lane & g) == 0, pltpu.roll(f, 128 - g, 1), pltpu.roll(f, g, 1))
            logits.append(f)
        if r0 < HALO:
            row = jax.lax.broadcasted_iota(jnp.int32, (n, 128), 0) + (row0 + r0)
            logits = [logits[0]] + [jnp.where(row >= DIL * w, logits[w], -1e9) for w in range(1, W)]
        m = logits[0]
        for w in range(1, W):
            m = jnp.maximum(m, logits[w])
        e = [jnp.exp2((logits[w] - m) * (DH ** -0.5 * LOG2E)) for w in range(W)]
        s = e[0]
        for w in range(1, W):
            s = s + e[w]
        r = gate[r0:r0 + n] * _recip(s)
        p = [e[w] * r for w in range(W)]
        o = []
        for t in range(NT):
            acc_o = None
            for w in range(W):
                x = p[w] * window(1, t, w, r0)
                acc_o = x if acc_o is None else acc_o + x
            o.append(acc_o)
        ou = _butterfly([pltpu.bitcast(x.astype(bf), jnp.uint32) for x in o], lane_h, reverse=True)
        for t in range(NT):
            ob_s[r0 // 2:(r0 + n) // 2, t * 128:(t + 1) * 128] = ou[t]

    points = [(c, k) for c in range(NCHUNK) for k in "gud"][3:]
    assign = {}
    for sb in range(NSLAB):
        assign.setdefault(points[(sb * len(points)) // NSLAB], []).append(sb)

    def run_slabs(c, k, m):
        for sb in assign.get((c, k), []):
            slab(sb * n, [m[0:n, 0:128], m[96:96 + n, 0:128], m[128:128 + n, 128:256]])

    acc = None
    for c in range(NCHUNK):
        g = jnp.dot(xa, wg_s[:, c * FC:(c + 1) * FC], preferred_element_type=f32)
        run_slabs(c, "g", g)
        u = jnp.dot(xa, wu_s[:, c * FC:(c + 1) * FC], preferred_element_type=f32)
        run_slabs(c, "u", u)
        h = (jax.nn.gelu(g, approximate=True) * u * omg).astype(bf)
        d = jnp.dot(h, wd_s[c * FC:(c + 1) * FC, :], preferred_element_type=f32)
        run_slabs(c, "d", d)
        acc = d if acc is None else acc + d
    ob = asbf(ob_s[...])
    slot = i % 2
    for g in range(OG):
        res = acc[:, g * OW:(g + 1) * OW] + jnp.dot(ob, wo_s[:, g * OW:(g + 1) * OW],
                                                     preferred_element_type=f32)
        obuf[slot, :, g * OW:(g + 1) * OW] = res.astype(bf)
        out_dma(i, g).start()

    @pl.when(i == NSTEPS - 1)
    def _():
        for g in range(OG):
            out_dma(i - 1, g).wait()
        for g in range(OG):
            out_dma(i, g).wait()


@jax.jit
def pallas_gated_mix__sliding_local_dilated__glu_gated_geglu__prompt_kernel(
    A_x: jax.Array,
    A_wqkv: jax.Array,
    A_wo: jax.Array,
    B_x: jax.Array,
    B_w_gate: jax.Array,
    B_w_up: jax.Array,
    B_w_down: jax.Array,
    gate_w: jax.Array,
):
    del B_x
    hbm = pl.BlockSpec(memory_space=pl.ANY)
    u32, bf16 = jnp.uint32, jnp.bfloat16
    out = pl.pallas_call(
        _kernel,
        grid=(NSTEPS,),
        in_specs=[hbm] * 7,
        out_specs=hbm,
        out_shape=jax.ShapeDtypeStruct((S, D), jnp.bfloat16),
        scratch_shapes=[
            pltpu.VMEM((S, D), bf16),
            pltpu.VMEM((D,), jnp.bfloat16),
            pltpu.VMEM((NQ, D, QC), bf16),
            pltpu.VMEM((D, D), bf16),
            pltpu.VMEM((D, DF), bf16),
            pltpu.VMEM((D, DF), bf16),
            pltpu.VMEM((DF, D), bf16),
            pltpu.VMEM((3 * NT, S, 128), jnp.float32),
            pltpu.VMEM((8 * NT, KR, 128), jnp.float32),
            pltpu.VMEM((TM // 2, D), u32),
            pltpu.VMEM((2, TM, D), jnp.bfloat16),
            pltpu.SemaphoreType.DMA((NSEMS,)),
        ],
        compiler_params=pltpu.CompilerParams(
            dimension_semantics=("arbitrary",), vmem_limit_bytes=120 * 1024 * 1024),
        name="fused",
    )(A_x.reshape(S, D), gate_w, A_wqkv, A_wo, B_w_gate, B_w_up, B_w_down)
    return out.reshape(1, S, D)
```
